```python
import os as _os
_os.environ.setdefault('JAX_PLATFORMS', 'cpu')
import jax
import jax.numpy as jnp

def _softmax(x, axis=-1):
    return jax.nn.softmax(x, axis=axis)

def _gelu(x):
    return jax.nn.gelu(x, approximate=True)

def _silu(x):
    return jax.nn.silu(x)

def _sigmoid(x):
    return jax.nn.sigmoid(x)

def _layernorm(x, axis=-1, eps=1e-05):
    m = jnp.mean(x, axis=axis, keepdims=True)
    v = jnp.var(x, axis=axis, keepdims=True)
    return (x - m) / jnp.sqrt(v + eps)

def _scatter_add(tgt, idx, src, axis=0):
    return tgt.at[idx].add(src)

def _segment_sum(src, seg, n):
    return jax.ops.segment_sum(src, seg, n)

class _Rng:

    def __init__(self, key):
        self._k = key

    def _next(self):
        self._k, sub = jax.random.split(self._k)
        return sub

    def normal(self, shape):
        return jax.random.normal(self._next(), shape, dtype=jnp.bfloat16)

    def randint(self, lo, hi, shape):
        return jax.random.randint(self._next(), shape, lo, hi, dtype=jnp.int32)

    def uniform(self, shape, lo=0.0, hi=1.0):
        return jax.random.uniform(self._next(), shape, jnp.bfloat16, lo, hi)

    def permutation(self, n):
        return jax.random.permutation(self._next(), n)
kernel_name = 'adaLN_cond__mha_block__dense_activation_squared_relu__prompt'

def setup_inputs():
    _rng = _Rng(jax.random.key(int.from_bytes(__import__("os").urandom(4), "little")))
    _w = lambda a: (lambda t: t.astype(jnp.bfloat16) if jnp.issubdtype(t.dtype, jnp.floating) else t)(jnp.asarray(a))

    def _A_setup():
        B, S, D, H = (1, 2048, 512, 32)
        return {'x': _w((lambda *s: _rng.normal(s) * 0.05)(B, S, D)), 'wqkv': _w((lambda *s: _rng.normal(s) * 0.1)(D, 3 * D)), 'wo': _w((lambda *s: _rng.normal(s) * 0.05)(D, D))}
    _A_in = _A_setup()

    def _B_setup():
        B, S, D, F = (1, 2048, 512, 1792)
        return {'x': _w((lambda *s: _rng.normal(s) * 0.05)(B, S, D)), 'w1': _w((lambda *s: _rng.normal(s) * 0.05)(D, F)), 'b1': _w((lambda *s: _rng.normal(s) * 0.05)(F)), 'w2': _w((lambda *s: _rng.normal(s) * 0.05)(F, D)), 'b2': _w((lambda *s: _rng.normal(s) * 0.05)(D))}
    _B_in = _B_setup()
    return {'A_x': _A_in['x'], 'A_wqkv': _A_in['wqkv'], 'A_wo': _A_in['wo'], 'B_x': _B_in['x'], 'B_w1': _B_in['w1'], 'B_b1': _B_in['b1'], 'B_w2': _B_in['w2'], 'B_b2': _B_in['b2'], 'c': _w((lambda *s: _rng.normal(s) * 0.05)(1, 512) * 8.0), 'w_mod': _w((lambda *s: _rng.normal(s) * 0.05)(512, 6 * 512) * 512 ** (-0.5) * 8.0)}

def reference(A_x, A_wqkv, A_wo, B_x, B_w1, B_b1, B_w2, B_b2, c, w_mod):

    def _A_ref(x, wqkv, wo):
        B, S, D = x.shape
        H = 32
        Dh = D // H
        qkv = (lambda x, *d: x.transpose(*d))((x @ wqkv).reshape(B, S, 3, H, Dh), 2, 0, 3, 1, 4)
        q, k, v = (qkv[0], qkv[1], qkv[2])
        scores = jnp.einsum('bhqd,bhkd->bhqk', q, k) * Dh ** (-0.5)
        p = _softmax(scores, axis=-1)
        o = jnp.einsum('bhqk,bhkd->bhqd', p, v)
        return (lambda x, *d: x.transpose(*d))(o, 0, 2, 1, 3).reshape(B, S, D) @ wo

    def _B_ref(x, w1, b1, w2, b2):
        h = jnp.einsum('bsd,df->bsf', x, w1) + b1
        zero = jnp.zeros_like(h)
        r = jnp.where(h > zero, h, zero)
        h = r * r
        out = jnp.einsum('bsf,fd->bsd', h, w2) + b2
        return out
    x = A_x
    mod = (_silu(c) @ w_mod).reshape(c.shape[0], 6, 1, -1)
    sa, ca, ga, sb, cb, gb = (mod[:, 0].copy(), mod[:, 1].copy(), mod[:, 2].copy(), mod[:, 3].copy(), mod[:, 4].copy(), mod[:, 5].copy())
    h = _layernorm(x, axis=-1) * (1 + ca) + sa
    x = x + ga * _A_ref(h, A_wqkv, A_wo)
    h = _layernorm(x, axis=-1) * (1 + cb) + sb
    x = x + gb * _B_ref(h, B_w1, B_b1, B_w2, B_b2)
    return x
```

```python
import functools

import jax
import jax.numpy as jnp
import jax.experimental.pallas as pl
import jax.experimental.pallas.tpu as pltpu
from jax import lax

F32 = jnp.float32
BF16 = jnp.bfloat16
NT = (((1,), (1,)), ((), ()))
TN = (((0,), (0,)), ((), ()))
LOG2E = 1.4426950408889634
EPS = 1e-5

H = 32
TK = 128
TQ = 512
RB = 512
DEP = 3


def _ln_mod(x, scale1p, shift):
    mu = jnp.mean(x, axis=-1, keepdims=True)
    xc = x - mu
    var = jnp.mean(xc * xc, axis=-1, keepdims=True)
    return xc * lax.rsqrt(var + EPS) * scale1p + shift


def _block_kernel(x_hbm, wqkv_hbm, wo_hbm, w1_hbm, b1_hbm, w2_hbm, b2_hbm, c_hbm, wmod_hbm,
                  out_hbm,
                  x_v, wqkv_v, wo_v, w1_v, b1_v, w2_v, b2_v, c_v, wmod_v, out_v,
                  wqt_v, wvt_v, qt_v, k_v, vt_v, ot_v, s0_v, s1_v, mod_v, sems, osems,
                  *, S, D):
    NQ = S // TQ
    NK = S // TK
    NR = S // RB
    NG = D // 128
    DH = D // H

    def cp(src, dst, i):
        return pltpu.make_async_copy(src, dst, sems.at[i])

    cp_c = cp(c_hbm, c_v, 0)
    cp_wm0 = cp(wmod_hbm.at[:, pl.ds(0, 2 * D)], wmod_v.at[:, pl.ds(0, 2 * D)], 1)
    cp_x = [cp(x_hbm.at[pl.ds(r * RB, RB)], x_v.at[pl.ds(r * RB, RB)], 2 + r) for r in range(NR)]
    cp_wqkv = cp(wqkv_hbm, wqkv_v, 2 + NR)
    cp_wm1 = cp(wmod_hbm.at[:, pl.ds(2 * D, 4 * D)], wmod_v.at[:, pl.ds(2 * D, 4 * D)], 3 + NR)
    cp_wo = cp(wo_hbm, wo_v, 4 + NR)
    cp_w1 = cp(w1_hbm, w1_v, 5 + NR)
    cp_b1 = cp(b1_hbm, b1_v, 6 + NR)
    cp_w2 = cp(w2_hbm, w2_v, 7 + NR)
    cp_b2 = cp(b2_hbm, b2_v, 8 + NR)
    cp_c.start()
    cp_wm0.start()
    cp_x[0].start()
    cp_wqkv.start()
    for r in range(1, NR):
        cp_x[r].start()
    cp_wm1.start()
    cp_wo.start()
    cp_w1.start()
    cp_b1.start()
    cp_w2.start()
    cp_b2.start()

    cp_c.wait()
    cp_wm0.wait()
    cc = c_v[...].astype(F32)
    sc = (cc * jax.nn.sigmoid(cc)).astype(BF16)
    sc8 = jnp.broadcast_to(sc, (16, D))
    m01 = jnp.dot(sc8, wmod_v[:, pl.ds(0, 2 * D)], preferred_element_type=F32)[0:1]
    m01 = m01.astype(BF16).astype(F32)
    sa = m01[:, 0:D]
    ca1 = 1.0 + m01[:, D:2 * D]

    cp_wqkv.wait()
    for j in range(NG):
        cs = pl.ds(j * 128, 128)
        wqt_v[cs, :] = wqkv_v[:, pl.ds(j * 128, 128)].astype(F32).T.astype(BF16)
        wvt_v[cs, :] = wqkv_v[:, pl.ds(2 * D + j * 128, 128)].astype(F32).T.astype(BF16)
    qscale = (DH ** -0.5) * LOG2E
    for r in range(NR):
        cp_x[r].wait()
        rows = pl.ds(r * RB, RB)
        h = _ln_mod(x_v[rows, :].astype(F32), ca1, sa).astype(BF16)
        kk = jnp.dot(h, wqkv_v[:, pl.ds(D, D)], preferred_element_type=F32).astype(BF16)
        for g in range(NG):
            k_v[g, rows, :] = kk[:, g * 128:(g + 1) * 128]
        qt = lax.dot_general(wqt_v[...], h, NT, preferred_element_type=F32)
        qt_v[r] = (qt * qscale).astype(BF16)
        vt_v[r] = lax.dot_general(wvt_v[...], h, NT, preferred_element_type=F32).astype(BF16)

    srefs = (s0_v, s1_v)
    row_id = lax.broadcasted_iota(jnp.int32, (128, TQ), 0)

    def masked_q(t):
        j = t // H
        hd = t % H
        g = hd // 8
        lo = (hd % 8) * DH
        q = qt_v[j, pl.ds(pl.multiple_of(g * 128, 128), 128), :]
        keep = (row_id >= lo) & (row_id < lo + DH)
        return jnp.where(keep, q, jnp.zeros_like(q)), g

    def qk_tile(qm, g, kt, slot, mx):
        s = jnp.dot(k_v[g, pl.ds(kt * TK, TK), :], qm, preferred_element_type=F32)
        srefs[slot][pl.ds(kt * TK, TK), :] = s
        return jnp.maximum(mx, jnp.max(s.reshape(TK // 8, 8, TQ), axis=0))

    def pv_tile(t, kt, slot, m, l, acc):
        hd = t % H
        s = srefs[slot][pl.ds(kt * TK, TK), :]
        p = jnp.exp2(s.reshape(TK // 8, 8, TQ) - m[None])
        l = l + jnp.sum(p, axis=0)
        per = RB // TK
        vt = vt_v[kt // per, pl.ds(pl.multiple_of(hd * DH, DH), DH), pl.ds((kt % per) * TK, TK)]
        acc = acc + jnp.dot(vt, p.reshape(TK, TQ).astype(BF16), preferred_element_type=F32)
        return l, acc

    def finish(t, l, acc):
        j = t // H
        hd = t % H
        inv = 1.0 / jnp.sum(l, axis=0, keepdims=True)
        ot_v[j, pl.ds(pl.multiple_of(hd * DH, DH), DH), :] = (acc * inv).astype(BF16)

    def col_max(mx):
        return jnp.broadcast_to(jnp.max(mx, axis=0, keepdims=True), (8, TQ))

    def step(t, mx, slot, t_dyn=None):
        m = col_max(mx)
        qm, g = masked_q(t + 1)
        nmx = jnp.full((8, TQ), -jnp.inf, F32)
        l = jnp.zeros((8, TQ), F32)
        acc = jnp.zeros((DH, TQ), F32)
        hist = []
        for kt in range(NK):
            nmx = qk_tile(qm, g, kt, 1 - slot, nmx)
            mm = m
            if kt >= DEP:
                mm = m + hist[kt - DEP] * 0.0
            l, acc = pv_tile(t, kt, slot, mm, l, acc)
            hist.append(acc[0:8])
        finish(t, l, acc)
        return nmx

    T = NQ * H
    qm, g = masked_q(0)
    mx = jnp.full((8, TQ), -jnp.inf, F32)
    for kt in range(NK):
        mx = qk_tile(qm, g, kt, 0, mx)

    def body(i, mx):
        mx = step(2 * i, mx, 0)
        return step(2 * i + 1, mx, 1)

    mx = lax.fori_loop(0, T // 2 - 1, body, mx)
    mx = step(T - 2, mx, 0)
    m = col_max(mx)
    l = jnp.zeros((8, TQ), F32)
    acc = jnp.zeros((DH, TQ), F32)
    for kt in range(NK):
        l, acc = pv_tile(T - 1, kt, 1, m, l, acc)
    finish(T - 1, l, acc)

    cp_wm1.wait()
    m25 = jnp.dot(sc8, wmod_v[:, pl.ds(2 * D, 4 * D)], preferred_element_type=F32)[0:1]
    m25 = m25.astype(BF16).astype(F32)
    ga = m25[:, 0:D]
    sb = m25[:, D:2 * D]
    cb1 = 1.0 + m25[:, 2 * D:3 * D]
    gb = m25[:, 3 * D:4 * D]
    cp_wo.wait()
    cp_w1.wait()
    cp_b1.wait()
    cp_w2.wait()
    cp_b2.wait()
    b1 = b1_v[...].astype(F32).reshape(1, -1)
    b2 = b2_v[...].astype(F32).reshape(1, -1)

    def out_copy(r):
        rows = pl.ds(r * RB, RB)
        return pltpu.make_async_copy(out_v.at[rows], out_hbm.at[rows], osems.at[r])

    for r in range(NR):
        rows = pl.ds(r * RB, RB)
        y = lax.dot_general(ot_v[r], wo_v[...], TN, preferred_element_type=F32)
        x1 = x_v[rows, :].astype(F32) + ga * y
        h2 = _ln_mod(x1, cb1, sb).astype(BF16)
        a = jnp.dot(h2, w1_v[...], preferred_element_type=F32) + b1
        a = jnp.maximum(a, 0.0)
        f = (a * a).astype(BF16)
        z = jnp.dot(f, w2_v[...], preferred_element_type=F32) + b2
        out_v[rows, :] = (x1 + gb * z).astype(out_v.dtype)
        out_copy(r).start()
    for r in range(NR):
        out_copy(r).wait()


@jax.jit
def pallas_adaLN_cond__mha_block__dense_activation_squared_relu__prompt_kernel(
    A_x: jax.Array,
    A_wqkv: jax.Array,
    A_wo: jax.Array,
    B_x: jax.Array,
    B_w1: jax.Array,
    B_b1: jax.Array,
    B_w2: jax.Array,
    B_b2: jax.Array,
    c: jax.Array,
    w_mod: jax.Array,
):
    del B_x
    _, S, D = A_x.shape
    F = B_w1.shape[1]
    NQ = S // TQ
    NR = S // RB
    NG = D // 128
    assert TQ == RB
    hbm = pl.BlockSpec(memory_space=pltpu.MemorySpace.HBM)
    dt = A_x.dtype
    scratch = [
        pltpu.VMEM((S, D), dt),
        pltpu.VMEM((D, 3 * D), A_wqkv.dtype),
        pltpu.VMEM((D, D), A_wo.dtype),
        pltpu.VMEM((D, F), B_w1.dtype),
        pltpu.VMEM((F,), B_b1.dtype),
        pltpu.VMEM((F, D), B_w2.dtype),
        pltpu.VMEM((D,), B_b2.dtype),
        pltpu.VMEM((1, D), c.dtype),
        pltpu.VMEM((D, 6 * D), w_mod.dtype),
        pltpu.VMEM((S, D), dt),
        pltpu.VMEM((D, D), BF16),
        pltpu.VMEM((D, D), BF16),
        pltpu.VMEM((NQ, D, TQ), BF16),
        pltpu.VMEM((NG, S, 128), BF16),
        pltpu.VMEM((NR, D, RB), BF16),
        pltpu.VMEM((NQ, D, TQ), BF16),
        pltpu.VMEM((S, TQ), F32),
        pltpu.VMEM((S, TQ), F32),
        pltpu.VMEM((8, 6 * D), F32),
        pltpu.SemaphoreType.DMA((9 + NR,)),
        pltpu.SemaphoreType.DMA((NR,)),
    ]
    out = pl.pallas_call(
        functools.partial(_block_kernel, S=S, D=D),
        out_shape=jax.ShapeDtypeStruct((S, D), dt),
        in_specs=[hbm] * 9,
        out_specs=hbm,
        scratch_shapes=scratch,
        compiler_params=pltpu.CompilerParams(vmem_limit_bytes=100 * 1024 * 1024),
    )(A_x.reshape(S, D), A_wqkv, A_wo, B_w1, B_b1, B_w2, B_b2, c, w_mod)
    return out.reshape(1, S, D)
```

```python
import functools

import jax
import jax.numpy as jnp
import jax.experimental.pallas as pl
import jax.experimental.pallas.tpu as pltpu
from jax import lax

F32 = jnp.float32
BF16 = jnp.bfloat16
U32 = jnp.uint32
NT = (((1,), (1,)), ((), ()))
TN = (((0,), (0,)), ((), ()))
LOG2E = 1.4426950408889634
EPS = 1e-5

H = 32
TK = 128
TQ = 512
RB = 512
SUB = 128
DEP = 3
LDEP = 2
UNR = 8


def _ln_mod(x, scale1p, shift):
    mu = jnp.mean(x, axis=-1, keepdims=True)
    xc = x - mu
    var = jnp.mean(xc * xc, axis=-1, keepdims=True)
    return xc * lax.rsqrt(var + EPS) * scale1p + shift


def _block_kernel(x_hbm, wqkv_hbm, wo_hbm, w1_hbm, b1_hbm, w2_hbm, b2_hbm, c_hbm, wmod_hbm,
                  out_hbm,
                  x_v, wqkv_v, wo_v, w1_v, b1_v, w2_v, b2_v, c_v, wmod_v, out_v,
                  wqt_v, wvt_v, qt_v, k_v, vt_v, ot_v, s0_v, s1_v, qm0_v, qm1_v, sems, osems,
                  *, S, D):
    NQ = S // TQ
    NK = S // TK
    NR = S // RB
    NG = D // 128
    DH = D // H
    NSUB = RB // SUB
    T = NQ * H

    def cp(src, dst, i):
        return pltpu.make_async_copy(src, dst, sems.at[i])

    def wcols(ref, j):
        return ref.at[:, pl.ds(j * D, D)]

    cp_c = cp(c_hbm, c_v, 0)
    cp_wm0 = cp(wmod_hbm.at[:, pl.ds(0, 2 * D)], wmod_v.at[:, pl.ds(0, 2 * D)], 1)
    cp_wq = cp(wcols(wqkv_hbm, 0), wcols(wqkv_v, 0), 2)
    cp_wk = cp(wcols(wqkv_hbm, 1), wcols(wqkv_v, 1), 3)
    cp_wv = cp(wcols(wqkv_hbm, 2), wcols(wqkv_v, 2), 4)
    cp_x0a = cp(x_hbm.at[pl.ds(0, SUB)], x_v.at[pl.ds(0, SUB)], 5)
    cp_x0b = cp(x_hbm.at[pl.ds(SUB, RB - SUB)], x_v.at[pl.ds(SUB, RB - SUB)], 6)
    cp_wm1 = cp(wmod_hbm.at[:, pl.ds(2 * D, 4 * D)], wmod_v.at[:, pl.ds(2 * D, 4 * D)], 7)
    cp_wo = cp(wo_hbm, wo_v, 8)
    cp_w1 = cp(w1_hbm, w1_v, 9)
    cp_b1 = cp(b1_hbm, b1_v, 10)
    cp_w2 = cp(w2_hbm, w2_v, 11)
    cp_b2 = cp(b2_hbm, b2_v, 12)

    def cp_x(r):
        rows = pl.ds(pl.multiple_of(r * RB, RB), RB)
        return pltpu.make_async_copy(x_hbm.at[rows], x_v.at[rows], sems.at[12 + r])

    for d in (cp_c, cp_wm0, cp_x0a, cp_wk, cp_wq, cp_wv, cp_x0b):
        d.start()
    for r in range(1, NR):
        cp_x(r).start()
    for d in (cp_wm1, cp_wo, cp_w1, cp_b1, cp_w2, cp_b2):
        d.start()

    cp_c.wait()
    cp_wm0.wait()
    cc = c_v[...].astype(F32)
    sc = jnp.broadcast_to((cc * jax.nn.sigmoid(cc)).astype(BF16), (16, D))
    m01 = jnp.dot(sc, wmod_v[:, pl.ds(0, 2 * D)], preferred_element_type=F32)[0:1]
    m01 = m01.astype(BF16).astype(F32)
    sa = m01[:, 0:D]
    ca1 = 1.0 + m01[:, D:2 * D]

    qscale = (DH ** -0.5) * LOG2E

    def transpose_w(j, dst):
        for i in range(NG):
            dst[pl.ds(i * 128, 128), :] = (
                wqkv_v[:, pl.ds(j * D + i * 128, 128)].astype(F32).T.astype(BF16))

    def ln1(r, i):
        rows = pl.ds(pl.multiple_of(r * RB + i * SUB, SUB), SUB)
        return _ln_mod(x_v[rows, :].astype(F32), ca1, sa).astype(BF16)

    def proj_k(r, i, h):
        rows2 = pl.ds(pl.multiple_of((r * RB + i * SUB) // 2, SUB // 2), SUB // 2)
        kk = jnp.dot(h, wqkv_v[:, pl.ds(D, D)], preferred_element_type=F32).astype(BF16)
        for g in range(NG):
            k_v[g, rows2, :] = pltpu.bitcast(kk[:, g * 128:(g + 1) * 128], U32)

    def proj_qt(r, i, h):
        qt = lax.dot_general(wqt_v[...], h, NT, preferred_element_type=F32)
        qt_v[r, :, pl.ds(i * SUB, SUB)] = pltpu.bitcast((qt * qscale).astype(BF16), U32)

    def proj_vt(r, i, h):
        vt = lax.dot_general(wvt_v[...], h, NT, preferred_element_type=F32)
        vt_v[r, :, pl.ds(i * SUB, SUB)] = pltpu.bitcast(vt.astype(BF16), U32)

    def proj_all(r, i, h):
        proj_k(r, i, h)
        proj_qt(r, i, h)
        proj_vt(r, i, h)

    cp_x0a.wait()
    h0 = ln1(0, 0)
    cp_wk.wait()
    proj_k(0, 0, h0)
    cp_wq.wait()
    transpose_w(0, wqt_v)
    proj_qt(0, 0, h0)
    cp_wv.wait()
    transpose_w(2, wvt_v)
    proj_vt(0, 0, h0)
    cp_x0b.wait()
    for i in range(1, NSUB):
        proj_all(0, i, ln1(0, i))
    cp_x(1).wait()

    def qkv_body(r, h_first):
        @pl.when(r + 1 < NR)
        def _():
            cp_x(r + 1).wait()

        proj_all(r, 0, h_first)
        for i in range(1, NSUB - 1):
            proj_all(r, i, ln1(r, i))
        h_last = ln1(r, NSUB - 1)
        h_next = ln1(jnp.minimum(r + 1, NR - 1), 0)
        proj_all(r, NSUB - 1, h_last)
        return h_next

    lax.fori_loop(1, NR, qkv_body, ln1(1, 0))

    srefs = (s0_v, s1_v)
    qrefs = (qm0_v, qm1_v)
    row_id = lax.broadcasted_iota(jnp.int32, (64, TQ), 0)
    neg_inf = jnp.full((8, TQ), -jnp.inf, F32)

    def stage_q(t, slot):
        j = t // H
        hd = t % H
        lo = (hd % 8) * (DH // 2)
        q = qt_v[j, pl.ds(pl.multiple_of((hd // 8) * 64, 64), 64), :]
        keep = (row_id >= lo) & (row_id < lo + DH // 2)
        qrefs[slot][...] = jnp.where(keep, q, jnp.zeros_like(q))

    def qk_tile(g, kt, slot, mx):
        kk = pltpu.bitcast(k_v[g, pl.ds(kt * (TK // 2), TK // 2), :], BF16)
        qm = pltpu.bitcast(qrefs[slot][...], BF16)
        s = jnp.dot(kk, qm, preferred_element_type=F32)
        srefs[slot][pl.ds(kt * TK, TK), :] = s
        return jnp.maximum(mx, jnp.max(s.reshape(TK // 8, 8, TQ), axis=0))

    def pv_tile(t, kt, slot, m, l, acc):
        hd = t % H
        s = srefs[slot][pl.ds(kt * TK, TK), :]
        p = jnp.exp2(s.reshape(TK // 8, 8, TQ) - m[None])
        for i in range(0, TK // 8, 2):
            l = l + (p[i] + p[i + 1])
        per = RB // TK
        vt = vt_v[kt // per, pl.ds(pl.multiple_of(hd * (DH // 2), DH // 2), DH // 2),
                  pl.ds((kt % per) * TK, TK)]
        acc = acc + jnp.dot(pltpu.bitcast(vt, BF16), p.reshape(TK, TQ).astype(BF16),
                            preferred_element_type=F32)
        return l, acc

    def finish(t, l, acc):
        inv = 1.0 / jnp.sum(l, axis=0, keepdims=True)
        ot_v[t // H, pl.ds(pl.multiple_of((t % H) * DH, DH), DH), :] = (acc * inv).astype(BF16)

    def col_max(mx):
        return jnp.broadcast_to(jnp.max(mx, axis=0, keepdims=True), (8, TQ))

    def step(t, m, nmx, slot, first_qk=True, last_qk=True):
        g1 = ((t + 1) % H) // 8
        g2 = ((t + 2) % H) // 8
        if last_qk:
            stage_q(t + 2, slot)
        l = jnp.zeros((8, TQ), F32)
        acc = jnp.zeros((DH, TQ), F32)
        hist = []
        lhist = []
        m_next = None
        for kt in range(NK):
            if kt < NK - 1:
                if first_qk:
                    nmx = qk_tile(g1, kt + 1, 1 - slot, nmx)
            else:
                if first_qk:
                    m_next = col_max(nmx)
                if last_qk:
                    nmx = qk_tile(g2, 0, slot, neg_inf)
            mm = m
            if kt >= DEP:
                mm = mm + hist[kt - DEP] * 0.0
            if kt >= LDEP:
                mm = mm + lhist[kt - LDEP] * 0.0
            l, acc = pv_tile(t, kt, slot, mm, l, acc)
            hist.append(acc[0:8])
            lhist.append(l)
        finish(t, l, acc)
        return m_next, nmx

    stage_q(0, 0)
    stage_q(1, 1)
    cp_wm1.wait()
    mx = neg_inf
    macc = [jnp.zeros((16, D), F32) for _ in range(4)]
    for kt in range(NK):
        mx = qk_tile(0, kt, 0, mx)
        n, kk = kt // NG, kt % NG
        macc[n] = macc[n] + jnp.dot(sc[:, kk * 128:(kk + 1) * 128],
                                    wmod_v[pl.ds(kk * 128, 128), pl.ds((2 + n) * D, D)],
                                    preferred_element_type=F32)
    ga, sb, cb, gb = [a[0:1].astype(BF16).astype(F32) for a in macc]
    cb1 = 1.0 + cb
    m = col_max(mx)
    nmx = qk_tile(0, 0, 1, neg_inf)

    def attn_body(i, carry):
        m, nmx = carry
        for u in range(UNR):
            m, nmx = step(UNR * i + u, m, nmx, u % 2)
        return m, nmx

    n_it = (T - 2) // UNR
    m, nmx = lax.fori_loop(0, n_it, attn_body, (m, nmx))
    for t in range(n_it * UNR, T - 2):
        m, nmx = step(t, m, nmx, t % 2)
    m, nmx = step(T - 2, m, nmx, 0, last_qk=False)
    step(T - 1, m, nmx, 1, first_qk=False, last_qk=False)

    cp_wo.wait()
    cp_w1.wait()
    cp_b1.wait()
    cp_w2.wait()
    cp_b2.wait()
    b1 = b1_v[...].astype(F32).reshape(1, -1)
    b2 = b2_v[...].astype(F32).reshape(1, -1)

    def out_copy(r, i):
        rows = pl.ds(pl.multiple_of(r * RB + i * SUB, SUB), SUB)
        return pltpu.make_async_copy(out_v.at[rows], out_hbm.at[rows], osems.at[r * NSUB + i])

    def mlp_body(r, carry):
        rws = [pl.ds(pl.multiple_of(r * RB + i * SUB, SUB), SUB) for i in range(NSUB)]
        ys = [lax.dot_general(ot_v[r, :, pl.ds(i * SUB, SUB)], wo_v[...], TN,
                              preferred_element_type=F32) for i in range(NSUB)]
        x1s = [x_v[rws[i], :].astype(F32) + ga * ys[i] for i in range(NSUB)]
        h2s = [_ln_mod(x1s[i], cb1, sb).astype(BF16) for i in range(NSUB)]
        fs = []
        for i in range(NSUB):
            a = jnp.dot(h2s[i], w1_v[...], preferred_element_type=F32) + b1
            a = jnp.maximum(a, 0.0)
            fs.append((a * a).astype(BF16))
        for i in range(NSUB):
            z = jnp.dot(fs[i], w2_v[...], preferred_element_type=F32) + b2
            out_v[rws[i], :] = (x1s[i] + gb * z).astype(out_v.dtype)
            out_copy(r, i).start()
        return carry

    lax.fori_loop(0, NR, mlp_body, 0)
    for r in range(NR):
        for i in range(NSUB):
            out_copy(r, i).wait()


@jax.jit
def pallas_adaLN_cond__mha_block__dense_activation_squared_relu__prompt_kernel(
    A_x: jax.Array,
    A_wqkv: jax.Array,
    A_wo: jax.Array,
    B_x: jax.Array,
    B_w1: jax.Array,
    B_b1: jax.Array,
    B_w2: jax.Array,
    B_b2: jax.Array,
    c: jax.Array,
    w_mod: jax.Array,
):
    del B_x
    _, S, D = A_x.shape
    F = B_w1.shape[1]
    NQ = S // TQ
    NR = S // RB
    NG = D // 128
    assert TQ == RB and D == 512 and S % RB == 0 and NR >= 2
    hbm = pl.BlockSpec(memory_space=pltpu.MemorySpace.HBM)
    dt = A_x.dtype
    scratch = [
        pltpu.VMEM((S, D), dt),
        pltpu.VMEM((D, 3 * D), A_wqkv.dtype),
        pltpu.VMEM((D, D), A_wo.dtype),
        pltpu.VMEM((D, F), B_w1.dtype),
        pltpu.VMEM((F,), B_b1.dtype),
        pltpu.VMEM((F, D), B_w2.dtype),
        pltpu.VMEM((D,), B_b2.dtype),
        pltpu.VMEM((1, D), c.dtype),
        pltpu.VMEM((D, 6 * D), w_mod.dtype),
        pltpu.VMEM((S, D), dt),
        pltpu.VMEM((D, D), BF16),
        pltpu.VMEM((D, D), BF16),
        pltpu.VMEM((NQ, D // 2, TQ), U32),
        pltpu.VMEM((NG, S // 2, 128), U32),
        pltpu.VMEM((NR, D // 2, RB), U32),
        pltpu.VMEM((NQ, D, TQ), BF16),
        pltpu.VMEM((S, TQ), F32),
        pltpu.VMEM((S, TQ), F32),
        pltpu.VMEM((64, TQ), U32),
        pltpu.VMEM((64, TQ), U32),
        pltpu.SemaphoreType.DMA((13 + NR,)),
        pltpu.SemaphoreType.DMA((NR * (RB // SUB),)),
    ]
    out = pl.pallas_call(
        functools.partial(_block_kernel, S=S, D=D),
        out_shape=jax.ShapeDtypeStruct((S, D), dt),
        in_specs=[hbm] * 9,
        out_specs=hbm,
        scratch_shapes=scratch,
        compiler_params=pltpu.CompilerParams(vmem_limit_bytes=100 * 1024 * 1024),
    )(A_x.reshape(S, D), A_wqkv, A_wo, B_w1, B_b1, B_w2, B_b2, c, w_mod)
    return out.reshape(1, S, D)
```

```python
import functools

import jax
import jax.numpy as jnp
import jax.experimental.pallas as pl
import jax.experimental.pallas.tpu as pltpu
from jax import lax

F32 = jnp.float32
BF16 = jnp.bfloat16
U32 = jnp.uint32
NT = (((1,), (1,)), ((), ()))
TN = (((0,), (0,)), ((), ()))
LOG2E = 1.4426950408889634
EPS = 1e-5

H = 32
TK = 128
TQ = 512
RB = 512
SUB = 128
DEP = 3
LDEP = 2
UNR = 14


def _ln_mod(x, scale1p, shift):
    mu = jnp.mean(x, axis=-1, keepdims=True)
    xc = x - mu
    var = jnp.mean(xc * xc, axis=-1, keepdims=True)
    return xc * lax.rsqrt(var + EPS) * scale1p + shift


def _block_kernel(x_hbm, wqkv_hbm, wo_hbm, w1_hbm, b1_hbm, w2_hbm, b2_hbm, c_hbm, wmod_hbm,
                  out_hbm,
                  x_v, wqkv_v, wo_v, w1_v, b1_v, w2_v, b2_v, c_v, wmod_v, out_v,
                  wqt_v, wvt_v, qt_v, k_v, vt_v, ot_v, s0_v, s1_v, qm0_v, qm1_v, sems, osems,
                  *, S, D):
    NQ = S // TQ
    NK = S // TK
    NR = S // RB
    NG = D // 128
    DH = D // H
    NSUB = RB // SUB
    T = NQ * H

    def cp(src, dst, i):
        return pltpu.make_async_copy(src, dst, sems.at[i])

    def wcols(ref, j):
        return ref.at[:, pl.ds(j * D, D)]

    cp_c = cp(c_hbm, c_v, 0)
    cp_wm0 = cp(wmod_hbm.at[:, pl.ds(0, 2 * D)], wmod_v.at[:, pl.ds(0, 2 * D)], 1)
    cp_wq = cp(wcols(wqkv_hbm, 0), wcols(wqkv_v, 0), 2)
    cp_wk = cp(wcols(wqkv_hbm, 1), wcols(wqkv_v, 1), 3)
    cp_wv = cp(wcols(wqkv_hbm, 2), wcols(wqkv_v, 2), 4)
    cp_x0a = cp(x_hbm.at[pl.ds(0, SUB)], x_v.at[pl.ds(0, SUB)], 5)
    cp_x0b = cp(x_hbm.at[pl.ds(SUB, RB - SUB)], x_v.at[pl.ds(SUB, RB - SUB)], 6)
    cp_wm1 = cp(wmod_hbm.at[:, pl.ds(2 * D, 4 * D)], wmod_v.at[:, pl.ds(2 * D, 4 * D)], 7)
    cp_wo = cp(wo_hbm, wo_v, 8)
    cp_w1 = cp(w1_hbm, w1_v, 9)
    cp_b1 = cp(b1_hbm, b1_v, 10)
    cp_w2 = cp(w2_hbm, w2_v, 11)
    cp_b2 = cp(b2_hbm, b2_v, 12)

    def cp_x(r):
        rows = pl.ds(pl.multiple_of(r * RB, RB), RB)
        return pltpu.make_async_copy(x_hbm.at[rows], x_v.at[rows], sems.at[12 + r])

    for d in (cp_c, cp_wm0, cp_x0a, cp_wk, cp_x0b, cp_wq, cp_wv):
        d.start()
    for r in range(1, NR):
        cp_x(r).start()
    for d in (cp_wm1, cp_wo, cp_w1, cp_b1, cp_w2, cp_b2):
        d.start()

    cp_c.wait()
    cp_wm0.wait()
    cc = c_v[...].astype(F32)
    sc = jnp.broadcast_to((cc * jax.nn.sigmoid(cc)).astype(BF16), (16, D))
    m01 = jnp.dot(sc, wmod_v[:, pl.ds(0, 2 * D)], preferred_element_type=F32)[0:1]
    m01 = m01.astype(BF16).astype(F32)
    sa = m01[:, 0:D]
    ca1 = 1.0 + m01[:, D:2 * D]

    qscale = (DH ** -0.5) * LOG2E

    def transpose_w(j, dst):
        for i in range(NG):
            dst[pl.ds(i * 128, 128), :] = (
                wqkv_v[:, pl.ds(j * D + i * 128, 128)].astype(F32).T.astype(BF16))

    def ln1(r, i):
        rows = pl.ds(pl.multiple_of(r * RB + i * SUB, SUB), SUB)
        return _ln_mod(x_v[rows, :].astype(F32), ca1, sa).astype(BF16)

    def proj_k(r, i, h):
        rows2 = pl.ds(pl.multiple_of((r * RB + i * SUB) // 2, SUB // 2), SUB // 2)
        kk = jnp.dot(h, wqkv_v[:, pl.ds(D, D)], preferred_element_type=F32).astype(BF16)
        for g in range(NG):
            k_v[g, rows2, :] = pltpu.bitcast(kk[:, g * 128:(g + 1) * 128], U32)

    def proj_qt(r, i, h):
        qt = lax.dot_general(wqt_v[...], h, NT, preferred_element_type=F32)
        qt_v[r, :, pl.ds(i * SUB, SUB)] = pltpu.bitcast((qt * qscale).astype(BF16), U32)

    def proj_vt(r, i, h):
        vt = lax.dot_general(wvt_v[...], h, NT, preferred_element_type=F32)
        vt_v[r, :, pl.ds(i * SUB, SUB)] = pltpu.bitcast(vt.astype(BF16), U32)

    def proj_all(r, i, h):
        proj_k(r, i, h)
        proj_qt(r, i, h)
        proj_vt(r, i, h)

    cp_x0a.wait()
    hs = [ln1(0, 0)]
    cp_wk.wait()
    proj_k(0, 0, hs[0])
    cp_x0b.wait()
    for i in range(1, NSUB):
        hs.append(ln1(0, i))
    for i in range(1, NSUB - 1):
        proj_k(0, i, hs[i])
    cp_wq.wait()
    transpose_w(0, wqt_v)
    proj_k(0, NSUB - 1, hs[NSUB - 1])
    for i in range(NSUB // 2):
        proj_qt(0, i, hs[i])
    cp_wv.wait()
    transpose_w(2, wvt_v)
    for i in range(NSUB // 2, NSUB):
        proj_qt(0, i, hs[i])
    for i in range(NSUB):
        proj_vt(0, i, hs[i])
    cp_x(1).wait()

    def qkv_body(r, h_first):
        @pl.when(r + 1 < NR)
        def _():
            cp_x(r + 1).wait()

        proj_all(r, 0, h_first)
        for i in range(1, NSUB - 1):
            proj_all(r, i, ln1(r, i))
        h_last = ln1(r, NSUB - 1)
        h_next = ln1(jnp.minimum(r + 1, NR - 1), 0)
        proj_all(r, NSUB - 1, h_last)
        return h_next

    lax.fori_loop(1, NR, qkv_body, ln1(1, 0))

    srefs = (s0_v, s1_v)
    qrefs = (qm0_v, qm1_v)
    neg_inf = jnp.full((8, TQ), -jnp.inf, F32)

    def stage_q(t, slot):
        j = t // H
        hd = t % H
        lo = (hd % 8) * (DH // 2)
        qrefs[slot][...] = jnp.zeros((64, TQ), U32)
        qrefs[slot][pl.ds(pl.multiple_of(lo, DH // 2), DH // 2), :] = (
            qt_v[j, pl.ds(pl.multiple_of(hd * (DH // 2), DH // 2), DH // 2), :])

    def qk_tile(g, kt, slot, mx):
        kk = pltpu.bitcast(k_v[g, pl.ds(kt * (TK // 2), TK // 2), :], BF16)
        qm = pltpu.bitcast(qrefs[slot][...], BF16)
        s = jnp.dot(kk, qm, preferred_element_type=F32)
        srefs[slot][pl.ds(kt * TK, TK), :] = s
        return jnp.maximum(mx, jnp.max(s.reshape(TK // 8, 8, TQ), axis=0))

    def pv_tile(t, kt, slot, m, l, acc):
        hd = t % H
        s = srefs[slot][pl.ds(kt * TK, TK), :]
        p = jnp.exp2(s.reshape(TK // 8, 8, TQ) - m[None])
        for i in range(0, TK // 8, 2):
            l = l + (p[i] + p[i + 1])
        per = RB // TK
        vt = vt_v[kt // per, pl.ds(pl.multiple_of(hd * (DH // 2), DH // 2), DH // 2),
                  pl.ds((kt % per) * TK, TK)]
        acc = acc + jnp.dot(pltpu.bitcast(vt, BF16), p.reshape(TK, TQ).astype(BF16),
                            preferred_element_type=F32)
        return l, acc

    def finish(t, l, acc):
        inv = 1.0 / jnp.sum(l, axis=0, keepdims=True)
        ot_v[t // H, pl.ds(pl.multiple_of((t % H) * DH, DH), DH), :] = (acc * inv).astype(BF16)

    def col_max(mx):
        return jnp.broadcast_to(jnp.max(mx, axis=0, keepdims=True), (8, TQ))

    def step(t, m, nmx, slot, first_qk=True, last_qk=True):
        g1 = ((t + 1) % H) // 8
        g2 = ((t + 2) % H) // 8
        if last_qk:
            stage_q(t + 2, slot)
        l = jnp.zeros((8, TQ), F32)
        acc = jnp.zeros((DH, TQ), F32)
        hist = []
        lhist = []
        m_next = None
        for kt in range(NK):
            if kt < NK - 1:
                if first_qk:
                    nmx = qk_tile(g1, kt + 1, 1 - slot, nmx)
            else:
                if first_qk:
                    m_next = col_max(nmx)
                if last_qk:
                    nmx = qk_tile(g2, 0, slot, neg_inf)
            mm = m
            if kt >= DEP:
                mm = mm + hist[kt - DEP] * 0.0
            if kt >= LDEP:
                mm = mm + lhist[kt - LDEP] * 0.0
            l, acc = pv_tile(t, kt, slot, mm, l, acc)
            hist.append(acc[0:8])
            lhist.append(l)
        finish(t, l, acc)
        return m_next, nmx

    stage_q(0, 0)
    stage_q(1, 1)
    cp_wm1.wait()
    mx = neg_inf
    macc = [jnp.zeros((16, D), F32) for _ in range(4)]
    for kt in range(NK):
        mx = qk_tile(0, kt, 0, mx)
        n, kk = kt // NG, kt % NG
        macc[n] = macc[n] + jnp.dot(sc[:, kk * 128:(kk + 1) * 128],
                                    wmod_v[pl.ds(kk * 128, 128), pl.ds((2 + n) * D, D)],
                                    preferred_element_type=F32)
    ga, sb, cb, gb = [a[0:1].astype(BF16).astype(F32) for a in macc]
    cb1 = 1.0 + cb
    m = col_max(mx)
    nmx = qk_tile(0, 0, 1, neg_inf)

    def attn_body(i, carry):
        m, nmx = carry
        for u in range(UNR):
            m, nmx = step(UNR * i + u, m, nmx, u % 2)
        return m, nmx

    n_it = (T - 2) // UNR
    m, nmx = lax.fori_loop(0, n_it, attn_body, (m, nmx))
    for t in range(n_it * UNR, T - 2):
        m, nmx = step(t, m, nmx, t % 2)
    m, nmx = step(T - 2, m, nmx, 0, last_qk=False)
    step(T - 1, m, nmx, 1, first_qk=False, last_qk=False)

    cp_wo.wait()
    cp_w1.wait()
    cp_b1.wait()
    cp_w2.wait()
    cp_b2.wait()
    b1 = b1_v[...].astype(F32).reshape(1, -1)
    b2 = b2_v[...].astype(F32).reshape(1, -1)

    def out_copy(r, i):
        rows = pl.ds(pl.multiple_of(r * RB + i * SUB, SUB), SUB)
        return pltpu.make_async_copy(out_v.at[rows], out_hbm.at[rows], osems.at[r * NSUB + i])

    def mlp_body(r, carry):
        rws = [pl.ds(pl.multiple_of(r * RB + i * SUB, SUB), SUB) for i in range(NSUB)]
        ys = [lax.dot_general(ot_v[r, :, pl.ds(i * SUB, SUB)], wo_v[...], TN,
                              preferred_element_type=F32) for i in range(NSUB)]
        x1s = [x_v[rws[i], :].astype(F32) + ga * ys[i] for i in range(NSUB)]
        h2s = [_ln_mod(x1s[i], cb1, sb).astype(BF16) for i in range(NSUB)]
        fs = []
        for i in range(NSUB):
            a = jnp.dot(h2s[i], w1_v[...], preferred_element_type=F32) + b1
            a = jnp.maximum(a, 0.0)
            fs.append((a * a).astype(BF16))
        for i in range(NSUB):
            z = jnp.dot(fs[i], w2_v[...], preferred_element_type=F32) + b2
            out_v[rws[i], :] = (x1s[i] + gb * z).astype(out_v.dtype)
            out_copy(r, i).start()
        return carry

    lax.fori_loop(0, NR, mlp_body, 0)
    for r in range(NR):
        for i in range(NSUB):
            out_copy(r, i).wait()


@jax.jit
def pallas_adaLN_cond__mha_block__dense_activation_squared_relu__prompt_kernel(
    A_x: jax.Array,
    A_wqkv: jax.Array,
    A_wo: jax.Array,
    B_x: jax.Array,
    B_w1: jax.Array,
    B_b1: jax.Array,
    B_w2: jax.Array,
    B_b2: jax.Array,
    c: jax.Array,
    w_mod: jax.Array,
):
    del B_x
    _, S, D = A_x.shape
    F = B_w1.shape[1]
    NQ = S // TQ
    NR = S // RB
    NG = D // 128
    assert TQ == RB and D == 512 and S % RB == 0 and NR >= 2
    hbm = pl.BlockSpec(memory_space=pltpu.MemorySpace.HBM)
    dt = A_x.dtype
    scratch = [
        pltpu.VMEM((S, D), dt),
        pltpu.VMEM((D, 3 * D), A_wqkv.dtype),
        pltpu.VMEM((D, D), A_wo.dtype),
        pltpu.VMEM((D, F), B_w1.dtype),
        pltpu.VMEM((F,), B_b1.dtype),
        pltpu.VMEM((F, D), B_w2.dtype),
        pltpu.VMEM((D,), B_b2.dtype),
        pltpu.VMEM((1, D), c.dtype),
        pltpu.VMEM((D, 6 * D), w_mod.dtype),
        pltpu.VMEM((S, D), dt),
        pltpu.VMEM((D, D), BF16),
        pltpu.VMEM((D, D), BF16),
        pltpu.VMEM((NQ, D // 2, TQ), U32),
        pltpu.VMEM((NG, S // 2, 128), U32),
        pltpu.VMEM((NR, D // 2, RB), U32),
        pltpu.VMEM((NQ, D, TQ), BF16),
        pltpu.VMEM((S, TQ), F32),
        pltpu.VMEM((S, TQ), F32),
        pltpu.VMEM((64, TQ), U32),
        pltpu.VMEM((64, TQ), U32),
        pltpu.SemaphoreType.DMA((13 + NR,)),
        pltpu.SemaphoreType.DMA((NR * (RB // SUB),)),
    ]
    out = pl.pallas_call(
        functools.partial(_block_kernel, S=S, D=D),
        out_shape=jax.ShapeDtypeStruct((S, D), dt),
        in_specs=[hbm] * 9,
        out_specs=hbm,
        scratch_shapes=scratch,
        compiler_params=pltpu.CompilerParams(vmem_limit_bytes=100 * 1024 * 1024),
    )(A_x.reshape(S, D), A_wqkv, A_wo, B_w1, B_b1, B_w2, B_b2, c, w_mod)
    return out.reshape(1, S, D)
```
